```python
import os as _os
_os.environ.setdefault("JAX_PLATFORMS", "cpu")
import jax
import jax.numpy as jnp

def _softmax(x, axis=-1):
    return jax.nn.softmax(x, axis=axis)
def _gelu(x):
    return jax.nn.gelu(x, approximate=True)
def _silu(x):
    return jax.nn.silu(x)
def _sigmoid(x):
    return jax.nn.sigmoid(x)
def _layernorm(x, axis=-1, eps=1e-5):
    m = jnp.mean(x, axis=axis, keepdims=True)
    v = jnp.var(x, axis=axis, keepdims=True)
    return (x - m) / jnp.sqrt(v + eps)
def _scatter_add(tgt, idx, src, axis=0):
    return tgt.at[idx].add(src)
def _segment_sum(src, seg, n):
    return jax.ops.segment_sum(src, seg, n)
class _Rng:
    def __init__(self, key):
        self._k = key
    def _next(self):
        self._k, sub = jax.random.split(self._k)
        return sub
    def normal(self, shape):
        return jax.random.normal(self._next(), shape, dtype=jnp.bfloat16)
    def randint(self, lo, hi, shape):
        return jax.random.randint(self._next(), shape, lo, hi, dtype=jnp.int32)
    def uniform(self, shape, lo=0.0, hi=1.0):
        return jax.random.uniform(self._next(), shape, jnp.bfloat16, lo, hi)
    def permutation(self, n):
        return jax.random.permutation(self._next(), n)


kernel_name = 'gated_mix__mha_block__dense_activation_mish__prompt'

def setup_inputs():
    _rng = _Rng(jax.random.key(int.from_bytes(__import__("os").urandom(4), "little")))
    _w = (lambda a: (lambda t: t.astype(jnp.bfloat16) if jnp.issubdtype(t.dtype, jnp.floating) else t)(jnp.asarray(a)))
    def _A_setup():
        B, S, D, H = 1, 2048, 640, 32
        return {
            "x": _w((lambda *s: _rng.normal(s) * 0.05)(B, S, D)),
            "wqkv": _w((lambda *s: _rng.normal(s) * 0.2)(D, 3 * D)),
            "wo": _w((lambda *s: _rng.normal(s) * 0.05)(D, D)),
        }
    _A_in = _A_setup()

    def _B_setup():
        B, S, D, F = 1, 2048, 640, 1536
        return {
            "x": _w((lambda *s: _rng.normal(s) * 0.05)(B, S, D)),
            "w1": _w((lambda *s: _rng.normal(s) * 0.8)(D, F) * (D ** -0.5)),
            "b1": _w((lambda *s: _rng.normal(s) * 0.05)(F)),
            "w2": _w((lambda *s: _rng.normal(s) * 0.05)(F, D) * (F ** -0.5)),
        }
    _B_in = _B_setup()

    return {
        "A_x": _A_in["x"],
        "A_wqkv": _A_in["wqkv"],
        "A_wo": _A_in["wo"],
        "B_x": _B_in["x"],
        "B_w1": _B_in["w1"],
        "B_b1": _B_in["b1"],
        "B_w2": _B_in["w2"],
        "gate_w": _w((lambda *s: _rng.normal(s) * 0.05)(640) * 16.0),
    }

def reference(A_x, A_wqkv, A_wo, B_x, B_w1, B_b1, B_w2, gate_w):
    def _A_ref(x, wqkv, wo):
        B, S, D = x.shape
        H = 32
        Dh = D // H
        qkv = (lambda x, *d: x.transpose(*d))((x @ wqkv).reshape(B, S, 3, H, Dh), 2, 0, 3, 1, 4)
        q, k, v = qkv[0], qkv[1], qkv[2]
        scores = jnp.einsum("bhqd,bhkd->bhqk", q, k) * (Dh ** -0.5)
        p = _softmax(scores, axis=-1)
        o = jnp.einsum("bhqk,bhkd->bhqd", p, v)
        return (lambda x, *d: x.transpose(*d))(o, 0, 2, 1, 3).reshape(B, S, D) @ wo

    def _B_ref(x, w1, b1, w2):
        h = jnp.einsum("bsd,df->bsf", x, w1) + b1
        sp = jnp.log1p(jnp.exp(-jnp.abs(h))) + jnp.where(h > 0, h, jnp.zeros_like(h))
        act = h * jnp.tanh(sp)
        return jnp.einsum("bsf,fd->bsd", act, w2)

    x = A_x
    g = _sigmoid((x * gate_w).sum(-1, keepdims=True))
    a = _A_ref(x, A_wqkv, A_wo)
    b = _B_ref(x, B_w1, B_b1, B_w2)
    return g * a + (1 - g) * b
```

```python
import jax
import jax.numpy as jnp
from jax import lax
import jax.experimental.pallas as pl
import jax.experimental.pallas.tpu as pltpu

S, D, H, DH, F = 2048, 640, 32, 20, 1536
NT = D // 128
LOG2E = 1.4426950408889634
QSCALE = (DH ** -0.5) * LOG2E
RC = 512

F32, BF16, I32 = jnp.float32, jnp.bfloat16, jnp.int32
NN = (((1,), (0,)), ((), ()))
NT_DIMS = (((1,), (1,)), ((), ()))
TN = (((0,), (0,)), ((), ()))


def _dot(a, b, dims=NN):
    return lax.dot_general(a, b, dims, preferred_element_type=F32)


def _kernel(x_ref, wqkv_ref, wo_ref, w1_ref, b1_ref, w2_ref, gw_ref, o_ref,
            k_s, qt_s, vt_s, ot_s):
    x = x_ref[...]
    for t in range(NT):
        k_s[t] = _dot(x, wqkv_ref[:, D + 128 * t:D + 128 * t + 128]).astype(BF16)
    lane = lax.broadcasted_iota(I32, (S, 128), 1)
    for t in range(NT - 1):
        k_s[NT + t] = jnp.where(lane >= 64, k_s[t], k_s[t + 1])
    wq_t = wqkv_ref[:, 0:D].T
    wv_t = wqkv_ref[:, 2 * D:3 * D].T
    for t in range(NT):
        q = _dot(wq_t[128 * t:128 * t + 128], x, NT_DIMS)
        qt_s[t] = (q * QSCALE).astype(BF16)
    v = _dot(wv_t, x, NT_DIMS)
    vt_s[...] = v.astype(BF16).astype(F32)
    ot_s[...] = jnp.zeros((D, S), F32)

    def head(h, good, true_max):
        c = h * DH
        t = c // 128
        a = c - t * 128
        straddle = a + DH > 128
        kidx = jnp.where(straddle, NT + t, t)
        t2 = jnp.minimum(t + 1, NT - 1)
        qa = pltpu.bitcast(qt_s[t], I32)
        qb = pltpu.bitcast(qt_s[t2], I32)
        r2 = 2 * lax.broadcasted_iota(I32, (64, S), 0)
        w = jnp.where((r2 >= a) & (r2 < a + DH), qa,
                      jnp.where(r2 < a + DH - 128, qb, 0))
        w = pltpu.bitcast(w, BF16)
        s = _dot(k_s[kidx], w)
        if true_max:
            s = s - jnp.max(s, axis=0, keepdims=True)
        p = jnp.exp2(s).astype(BF16)
        g8 = pl.multiple_of((c // 8) * 8, 8)
        o = c - g8
        row = lax.broadcasted_iota(I32, (24, S), 0)
        lrow = jnp.where(o == 0, DH, 0)
        vt = jnp.where(row == lrow, 1.0, vt_s[pl.ds(g8, 24), :])
        acc = _dot(vt, p)
        l = jnp.sum(jnp.where(row == lrow, acc, 0.0), axis=0, keepdims=True)
        if not true_max:
            ok = (l >= 2.0 ** -60) & (l <= 2.0 ** 60)
            ok = ok & (jnp.max(jnp.abs(acc), axis=0, keepdims=True) <= 2.0 ** 120) & (
                jnp.min(jnp.where(jnp.abs(acc) <= 2.0 ** 120, 1.0, 0.0), axis=0, keepdims=True) > 0.5)
            good = jnp.minimum(good, jnp.where(ok, 1.0, 0.0))
        onorm = acc * (1.0 / l)
        keep = (row >= o) & (row < o + DH)
        ot_s[pl.ds(g8, 24), :] = jnp.where(keep, onorm, ot_s[pl.ds(g8, 24), :])
        return good

    good = lax.fori_loop(0, H, lambda h, g: head(h, g, False), jnp.ones((1, S), F32))

    @pl.when(jnp.min(good) < 0.5)
    def _():
        lax.fori_loop(0, H, lambda h, g: head(h, g, True), 0)

    gw = gw_ref[...].astype(F32)
    b1 = b1_ref[...].astype(F32)

    def rows(i, _):
        r0 = pl.multiple_of(i * RC, RC)
        xc = x_ref[pl.ds(r0, RC), :]
        g = jax.nn.sigmoid(jnp.sum(xc.astype(F32) * gw, axis=-1, keepdims=True))
        a = _dot(ot_s[:, pl.ds(r0, RC)].astype(BF16), wo_ref[...], TN)
        hh = _dot(xc, w1_ref[...]) + b1
        e = jnp.exp(jnp.minimum(hh, 20.0))
        n = e * (e + 2.0)
        act = (hh * (n / (n + 2.0))).astype(BF16)
        b = _dot(act, w2_ref[...])
        o_ref[pl.ds(r0, RC), :] = (g * a + (1.0 - g) * b).astype(o_ref.dtype)
        return _

    lax.fori_loop(0, S // RC, rows, 0)


@jax.jit
def pallas_gated_mix__mha_block__dense_activation_mish__prompt_kernel(
    A_x: jax.Array,
    A_wqkv: jax.Array,
    A_wo: jax.Array,
    B_x: jax.Array,
    B_w1: jax.Array,
    B_b1: jax.Array,
    B_w2: jax.Array,
    gate_w: jax.Array,
):
    del B_x
    out = pl.pallas_call(
        _kernel,
        out_shape=jax.ShapeDtypeStruct((S, D), A_x.dtype),
        scratch_shapes=[
            pltpu.VMEM((2 * NT - 1, S, 128), BF16),
            pltpu.VMEM((NT, 128, S), BF16),
            pltpu.VMEM((D, S), F32),
            pltpu.VMEM((D, S), F32),
        ],
        compiler_params=pltpu.CompilerParams(vmem_limit_bytes=110 * 1024 * 1024),
    )(A_x.reshape(S, D), A_wqkv, A_wo, B_w1, B_b1.reshape(1, F), B_w2, gate_w.reshape(1, D))
    return out.reshape(1, S, D)
```

```python
import jax
import jax.numpy as jnp
from jax import lax
import jax.experimental.pallas as pl
import jax.experimental.pallas.tpu as pltpu

S, D, H, DH, F = 2048, 640, 32, 20, 1536
NT = D // 128
LOG2E = 1.4426950408889634
QSCALE = (DH ** -0.5) * LOG2E
XC = 512
NXC = S // XC
QB, KB, AHEAD = 512, 128, 6
RC = 512
NRC = S // RC

F32, BF16, I32 = jnp.float32, jnp.bfloat16, jnp.int32
NN = (((1,), (0,)), ((), ()))
NT_DIMS = (((1,), (1,)), ((), ()))
TN = (((0,), (0,)), ((), ()))


def _dot(a, b, dims=NN):
    return lax.dot_general(a, b, dims, preferred_element_type=F32)


def _kernel(x_hbm, wqkv_hbm, wo_hbm, w1_hbm, b1_hbm, w2_hbm, gw_hbm, o_hbm,
            x_s, wq_s, wk_s, wv_s, wo_s, w1_s, b1_s, w2_s, gw_s, out_s,
            wt_s, k_s, vt_s, ot_s, w_s, in_sem, out_sem):
    def cp(src, dst, i):
        return pltpu.make_async_copy(src, dst, in_sem.at[i])

    x_cp = [cp(x_hbm.at[pl.ds(c * XC, XC), :], x_s.at[pl.ds(c * XC, XC), :], c)
            for c in range(NXC)]
    wq_cp = cp(wqkv_hbm.at[:, pl.ds(0, D)], wq_s, NXC)
    wk_cp = cp(wqkv_hbm.at[:, pl.ds(D, D)], wk_s, NXC + 1)
    wv_cp = cp(wqkv_hbm.at[:, pl.ds(2 * D, D)], wv_s, NXC + 2)
    late = [cp(wo_hbm, wo_s, NXC + 3), cp(w1_hbm, w1_s, NXC + 4), cp(w2_hbm, w2_s, NXC + 5),
            cp(b1_hbm, b1_s, NXC + 6), cp(gw_hbm, gw_s, NXC + 7)]

    def proj_k(c, extra=()):
        rows = pl.ds(c * XC, XC)
        lane = lax.broadcasted_iota(I32, (XC, 128), 1)
        xc = x_s[rows, :]
        k = []
        for t in range(NT):
            k.append(_dot(xc, wk_s[:, 128 * t:128 * t + 128]).astype(BF16))
            k_s[t, rows, :] = k[t]
            if t:
                k_s[NT + t - 1, rows, :] = jnp.where(lane >= 64, k[t - 1], k[t])
            for fn in extra:
                fn(t)

    def proj_qv(c, good):
        cols = pl.ds(pl.multiple_of(c * XC, XC), XC)
        qv = _dot(wt_s[...], x_s[cols, :], NT_DIMS)
        vt_s[:, cols] = qv[D:].astype(BF16).astype(F32)
        small = jnp.where(jnp.abs(qv[D:]) <= 2.0 ** 50, 1.0, 0.0)
        good = jnp.minimum(good, jnp.min(small, axis=0, keepdims=True))
        r = lax.broadcasted_iota(I32, (16, XC), 0)
        for h in range(H):
            lo, hi = DH * h, DH * h + DH
            for i in range(8):
                g0 = next((g for g in range(lo // 16 * 16, hi, 16) if g % 128 == 16 * i), None)
                if g0 is not None:
                    keep = (r >= lo - g0) & (r < hi - g0)
                    q = jnp.where(keep, qv[g0:g0 + 16] * QSCALE, 0.0)
                    w_s[h, 16 * i:16 * i + 16, cols] = q.astype(BF16)
        return good

    half = NXC // 2
    wk_cp.start()
    x_cp[0].start()
    for h in range(H):
        live = {g % 128 // 16 for g in range(DH * h // 16 * 16, DH * h + DH, 16)}
        for i in range(8):
            if i not in live:
                w_s[h, 16 * i:16 * i + 16, :] = jnp.zeros((16, S), BF16)
    wk_cp.wait()
    x_cp[0].wait()
    for c in range(1, half):
        x_cp[c].start()
    wq_cp.start()
    wv_cp.start()
    for c in range(half, NXC):
        x_cp[c].start()
    proj_k(0)
    for c in range(1, half):
        x_cp[c].wait()
        proj_k(c)
    wq_cp.wait()
    wv_cp.wait()
    for c in range(half, NXC):
        x_cp[c].wait()
    for c in late:
        c.start()
    slabs = [(w, r, t) for w, r in ((wq_s, 0), (wv_s, D)) for t in range(NT)]

    def transpose_slab(i):
        w, r, t = slabs[i]
        wt_s[r + 128 * t:r + 128 * t + 128, :] = w[:, 128 * t:128 * t + 128].T

    for c in range(half, NXC):
        proj_k(c, [lambda t, c=c: transpose_slab((c - half) * NT + t)])
    good = lax.fori_loop(0, NXC, proj_qv, jnp.ones((1, XC), F32))

    def head_fns(i, u):
        h = i * 2 + u
        c = h * DH
        t = c // 128
        kidx = jnp.where(c - t * 128 + DH > 128, NT + t, t)
        g8 = pl.multiple_of(i * (2 * DH) + u * 16, 8)
        lrow = 0 if u else DH
        row = lax.broadcasted_iota(I32, (24, KB), 0)
        row8 = lax.broadcasted_iota(I32, (8, QB), 0)

        def qk(g, j):
            return _dot(k_s[kidx, pl.ds(j * KB, KB), :], w_s[h, :, pl.ds(g * QB, QB)])

        def vt(j):
            return jnp.where(row == lrow, 1.0, vt_s[pl.ds(g8, 24), pl.ds(j * KB, KB)])

        def finish(g, acc, good):
            cols = pl.ds(g * QB, QB)
            l = acc[lrow:lrow + 1]
            r = pl.reciprocal(l, approx=True)
            o = acc * (r * (2.0 - l * r))
            if u:
                ot_s[pl.ds(g8, 8), cols] = jnp.where(row8 >= 4, o[:8], ot_s[pl.ds(g8, 8), cols])
                ot_s[pl.ds(g8 + 8, 16), cols] = o[8:]
            else:
                ot_s[pl.ds(g8, 24), cols] = o
            return jnp.minimum(good, jnp.where((l >= 2.0 ** -60) & (l <= 2.0 ** 60), 1.0, 0.0))

        return qk, vt, finish

    def heads_fast(i, good):
        fns = [head_fns(i, u) for u in range(2)]
        segs = [(u, g, j) for u in range(2) for g in range(S // QB) for j in range(S // KB)]
        pend = [fns[u][0](g, j) for u, g, j in segs[:AHEAD]]
        acc = None
        for n, (u, g, j) in enumerate(segs):
            if n + AHEAD < len(segs):
                u2, g2, j2 = segs[n + AHEAD]
                pend.append(fns[u2][0](g2, j2))
            d = _dot(fns[u][1](j), jnp.exp2(pend.pop(0)).astype(BF16))
            acc = d if j == 0 else acc + d
            if j == S // KB - 1:
                good = fns[u][2](g, acc, good)
        return good

    def tile_true_max(i, _):
        h = i // (S // 128)
        q0 = pl.multiple_of((i % (S // 128)) * 128, 128)
        c = h * DH
        t = c // 128
        kidx = jnp.where(c - t * 128 + DH > 128, NT + t, t)
        g8 = pl.multiple_of((c // 8) * 8, 8)
        o = c - g8
        lrow = jnp.where(o == 0, DH, 0)
        row = lax.broadcasted_iota(I32, (24, 128), 0)

        def qk(j):
            k0 = pl.multiple_of(j * KB, KB)
            return _dot(k_s[kidx, pl.ds(k0, KB), :], w_s[h, :, pl.ds(q0, 128)])

        m = lax.fori_loop(
            0, S // KB, lambda j, m: jnp.maximum(m, jnp.max(qk(j), axis=0, keepdims=True)),
            jnp.full((1, 128), -jnp.inf, F32))

        def pv(j, acc):
            v = vt_s[pl.ds(g8, 24), pl.ds(pl.multiple_of(j * KB, KB), KB)]
            return acc + _dot(jnp.where(row == lrow, 1.0, v), jnp.exp2(qk(j) - m).astype(BF16))

        acc = lax.fori_loop(0, S // KB, pv, jnp.zeros((24, 128), F32))
        l = jnp.sum(jnp.where(row == lrow, acc, 0.0), axis=0, keepdims=True)
        keep = (row >= o) & (row < o + DH)
        dst = ot_s.at[pl.ds(g8, 24), pl.ds(q0, 128)]
        dst[...] = jnp.where(keep, acc * (1.0 / l), dst[...])
        return _

    good = lax.fori_loop(0, H // 2, heads_fast, good)

    @pl.when(jnp.min(good) < 0.5)
    def _():
        lax.fori_loop(0, H * (S // 128), tile_true_max, 0)

    for c in late:
        c.wait()
    gw = gw_s[...].reshape(1, D).astype(F32)
    b1 = b1_s[...].reshape(1, F).astype(F32)

    def out_cp(i):
        rows = pl.ds(pl.multiple_of(i * RC, RC), RC)
        return pltpu.make_async_copy(out_s.at[rows, :], o_hbm.at[rows, :], out_sem.at[i])

    def rows_fn(i, _):
        r0 = pl.multiple_of(i * RC, RC)
        xc = x_s[pl.ds(r0, RC), :]
        g = jax.nn.sigmoid(jnp.sum(xc.astype(F32) * gw, axis=-1, keepdims=True))
        hh = _dot(xc, w1_s[...]) + b1
        a = _dot(ot_s[:, pl.ds(r0, RC)].astype(BF16), wo_s[...], TN)
        e = jnp.exp(jnp.minimum(hh, 20.0))
        n = e * (e + 2.0)
        act = (hh * (n / (n + 2.0))).astype(BF16)
        b = _dot(act, w2_s[...])
        out_s[pl.ds(r0, RC), :] = (g * a + (1.0 - g) * b).astype(BF16)
        out_cp(i).start()
        return _

    lax.fori_loop(0, NRC, rows_fn, 0)
    for i in range(NRC):
        out_cp(i).wait()


@jax.jit
def pallas_gated_mix__mha_block__dense_activation_mish__prompt_kernel(
    A_x: jax.Array,
    A_wqkv: jax.Array,
    A_wo: jax.Array,
    B_x: jax.Array,
    B_w1: jax.Array,
    B_b1: jax.Array,
    B_w2: jax.Array,
    gate_w: jax.Array,
):
    del B_x
    hbm = pl.BlockSpec(memory_space=pl.ANY)
    out = pl.pallas_call(
        _kernel,
        out_shape=jax.ShapeDtypeStruct((S, D), A_x.dtype),
        in_specs=[hbm] * 7,
        out_specs=hbm,
        scratch_shapes=[
            pltpu.VMEM((S, D), BF16),
            pltpu.VMEM((D, D), BF16),
            pltpu.VMEM((D, D), BF16),
            pltpu.VMEM((D, D), BF16),
            pltpu.VMEM((D, D), BF16),
            pltpu.VMEM((D, F), BF16),
            pltpu.VMEM((F,), BF16),
            pltpu.VMEM((F, D), BF16),
            pltpu.VMEM((D,), BF16),
            pltpu.VMEM((S, D), BF16),
            pltpu.VMEM((2 * D, D), BF16),
            pltpu.VMEM((2 * NT - 1, S, 128), BF16),
            pltpu.VMEM((D, S), F32),
            pltpu.VMEM((D, S), F32),
            pltpu.VMEM((H, 128, S), BF16),
            pltpu.SemaphoreType.DMA((NXC + 8,)),
            pltpu.SemaphoreType.DMA((NRC,)),
        ],
        compiler_params=pltpu.CompilerParams(vmem_limit_bytes=110 * 1024 * 1024),
    )(A_x.reshape(S, D), A_wqkv, A_wo, B_w1, B_b1, B_w2, gate_w)
    return out.reshape(1, S, D)
```

```python
import jax
import jax.numpy as jnp
from jax import lax
import jax.experimental.pallas as pl
import jax.experimental.pallas.tpu as pltpu

S, D, H, DH, F = 2048, 640, 32, 20, 1536
NT = D // 128
LOG2E = 1.4426950408889634
QSCALE = (DH ** -0.5) * LOG2E
XC = 512
NXC = S // XC
QB, KB, AHEAD = 512, 128, 6
assert XC == QB
RC = 512
NRC = S // RC

F32, BF16, I32 = jnp.float32, jnp.bfloat16, jnp.int32
NN = (((1,), (0,)), ((), ()))
NT_DIMS = (((1,), (1,)), ((), ()))
TN = (((0,), (0,)), ((), ()))


def _dot(a, b, dims=NN):
    return lax.dot_general(a, b, dims, preferred_element_type=F32)


def _kernel(x_hbm, wqkv_hbm, wo_hbm, w1_hbm, b1_hbm, w2_hbm, gw_hbm, o_hbm,
            x_s, wq_s, wk_s, wv_s, wo_s, w1_s, b1_s, w2_s, gw_s, out_s,
            wt_s, k_s, vt_s, ot_s, w_s, in_sem, out_sem):
    def cp(src, dst, i):
        return pltpu.make_async_copy(src, dst, in_sem.at[i])

    x_cp = [cp(x_hbm.at[pl.ds(c * XC, XC), :], x_s.at[pl.ds(c * XC, XC), :], c)
            for c in range(NXC)]
    wq_cp = cp(wqkv_hbm.at[:, pl.ds(0, D)], wq_s, NXC)
    wk_cp = cp(wqkv_hbm.at[:, pl.ds(D, D)], wk_s, NXC + 1)
    wv_cp = cp(wqkv_hbm.at[:, pl.ds(2 * D, D)], wv_s, NXC + 2)
    late = [cp(wo_hbm, wo_s, NXC + 3), cp(w1_hbm, w1_s, NXC + 4), cp(w2_hbm, w2_s, NXC + 5),
            cp(b1_hbm, b1_s, NXC + 6), cp(gw_hbm, gw_s, NXC + 7)]

    def proj_k(c, extra=()):
        rows = pl.ds(c * XC, XC)
        lane = lax.broadcasted_iota(I32, (XC, 128), 1)
        xc = x_s[rows, :]
        k = []
        for t in range(NT):
            parts = 4 if t == NT - 1 else 1
            w = wk_s[:, 128 * t:128 * t + 128]
            k.append(jnp.concatenate(
                [_dot(xc[i * XC // parts:(i + 1) * XC // parts], w) for i in range(parts)],
                axis=0).astype(BF16))
            k_s[t, rows, :] = k[t]
            if t:
                k_s[NT + t - 1, rows, :] = jnp.where(lane >= 64, k[t - 1], k[t])
            for fn in extra:
                fn(t)

    def proj_qv(c, good):
        cols = pl.ds(pl.multiple_of(c * XC, XC), XC)
        qv = _dot(wt_s[...], x_s[cols, :], NT_DIMS)
        vt_s[:, cols] = qv[D:].astype(BF16).astype(F32)
        small = jnp.where(jnp.abs(qv[D:]) <= 2.0 ** 50, 1.0, 0.0)
        good = jnp.minimum(good, jnp.min(small, axis=0, keepdims=True))
        r = lax.broadcasted_iota(I32, (16, XC), 0)
        for h in range(H):
            lo, hi = DH * h, DH * h + DH
            for i in range(8):
                g0 = next((g for g in range(lo // 16 * 16, hi, 16) if g % 128 == 16 * i), None)
                if g0 is not None:
                    keep = (r >= lo - g0) & (r < hi - g0)
                    q = jnp.where(keep, qv[g0:g0 + 16] * QSCALE, 0.0)
                    w_s[h, 16 * i:16 * i + 16, cols] = q.astype(BF16)
        return good

    half = NXC // 2
    wk_cp.start()
    x_cp[0].start()
    for h in range(H):
        live = {g % 128 // 16 for g in range(DH * h // 16 * 16, DH * h + DH, 16)}
        for i in range(8):
            if i not in live:
                w_s[h, 16 * i:16 * i + 16, :] = jnp.zeros((16, S), BF16)
    wk_cp.wait()
    x_cp[0].wait()
    for c in range(1, half):
        x_cp[c].start()
    wq_cp.start()
    wv_cp.start()
    for c in range(half, NXC):
        x_cp[c].start()
    proj_k(0)
    for c in range(1, half):
        x_cp[c].wait()
        proj_k(c)
    wq_cp.wait()
    wv_cp.wait()
    for c in range(half, NXC):
        x_cp[c].wait()
    for c in late:
        c.start()
    slabs = [(w, r, t) for w, r in ((wq_s, 0), (wv_s, D)) for t in range(NT)]

    def transpose_slab(i):
        w, r, t = slabs[i]
        wt_s[r + 128 * t:r + 128 * t + 128, :] = w[:, 128 * t:128 * t + 128].T

    for c in range(half, NXC):
        proj_k(c, [lambda t, c=c: transpose_slab((c - half) * NT + t)])
    good = lax.fori_loop(0, NXC, proj_qv, jnp.ones((1, XC), F32))

    def head_fns(i, u):
        h = i * 2 + u
        c = h * DH
        t = c // 128
        kidx = jnp.where(c - t * 128 + DH > 128, NT + t, t)
        g8 = pl.multiple_of(i * (2 * DH) + u * 16, 8)
        lrow = 0 if u else DH
        row = lax.broadcasted_iota(I32, (24, KB), 0)
        row8 = lax.broadcasted_iota(I32, (8, QB), 0)

        def qk(g, j):
            return _dot(k_s[kidx, pl.ds(j * KB, KB), :], w_s[h, :, pl.ds(g * QB, QB)])

        def vt(j):
            return jnp.where(row == lrow, 1.0, vt_s[pl.ds(g8, 24), pl.ds(j * KB, KB)])

        def finish(g, acc, good):
            cols = pl.ds(g * QB, QB)
            l = acc[lrow:lrow + 1]
            r = pl.reciprocal(l, approx=True)
            o = acc * (r * (2.0 - l * r))
            if u:
                ot_s[pl.ds(g8, 8), cols] = jnp.where(row8 >= 4, o[:8], ot_s[pl.ds(g8, 8), cols])
                ot_s[pl.ds(g8 + 8, 16), cols] = o[8:]
            else:
                ot_s[pl.ds(g8, 24), cols] = o
            return jnp.minimum(good, jnp.where((l >= 2.0 ** -60) & (l <= 2.0 ** 60), 1.0, 0.0))

        return qk, vt, finish

    def heads_fast(i, good):
        fns = [head_fns(i, u) for u in range(2)]
        segs = [(u, g, j) for u in range(2) for g in range(S // QB) for j in range(S // KB)]
        pend = [fns[u][0](g, j) for u, g, j in segs[:AHEAD]]
        acc = None
        for n, (u, g, j) in enumerate(segs):
            if n + AHEAD < len(segs):
                u2, g2, j2 = segs[n + AHEAD]
                pend.append(fns[u2][0](g2, j2))
            d = _dot(fns[u][1](j), jnp.exp2(pend.pop(0)).astype(BF16))
            acc = d if j == 0 else acc + d
            if j == S // KB - 1:
                good = fns[u][2](g, acc, good)
        return good

    def tile_true_max(i, _):
        h = i // (S // 128)
        q0 = pl.multiple_of((i % (S // 128)) * 128, 128)
        c = h * DH
        t = c // 128
        kidx = jnp.where(c - t * 128 + DH > 128, NT + t, t)
        g8 = pl.multiple_of((c // 8) * 8, 8)
        o = c - g8
        lrow = jnp.where(o == 0, DH, 0)
        row = lax.broadcasted_iota(I32, (24, 128), 0)

        def qk(j):
            k0 = pl.multiple_of(j * KB, KB)
            return _dot(k_s[kidx, pl.ds(k0, KB), :], w_s[h, :, pl.ds(q0, 128)])

        m = lax.fori_loop(
            0, S // KB, lambda j, m: jnp.maximum(m, jnp.max(qk(j), axis=0, keepdims=True)),
            jnp.full((1, 128), -jnp.inf, F32))

        def pv(j, acc):
            v = vt_s[pl.ds(g8, 24), pl.ds(pl.multiple_of(j * KB, KB), KB)]
            return acc + _dot(jnp.where(row == lrow, 1.0, v), jnp.exp2(qk(j) - m).astype(BF16))

        acc = lax.fori_loop(0, S // KB, pv, jnp.zeros((24, 128), F32))
        l = jnp.sum(jnp.where(row == lrow, acc, 0.0), axis=0, keepdims=True)
        keep = (row >= o) & (row < o + DH)
        dst = ot_s.at[pl.ds(g8, 24), pl.ds(q0, 128)]
        dst[...] = jnp.where(keep, acc * (1.0 / l), dst[...])
        return _

    good = lax.fori_loop(0, H // 2, heads_fast, good)

    @pl.when(jnp.min(good) < 0.5)
    def _():
        lax.fori_loop(0, H * (S // 128), tile_true_max, 0)

    for c in late:
        c.wait()
    gw = gw_s[...].reshape(1, D).astype(F32)
    b1 = b1_s[...].reshape(1, F).astype(F32)

    def out_cp(i):
        rows = pl.ds(pl.multiple_of(i * RC, RC), RC)
        return pltpu.make_async_copy(out_s.at[rows, :], o_hbm.at[rows, :], out_sem.at[i])

    def rows_fn(i, _):
        r0 = pl.multiple_of(i * RC, RC)
        xc = x_s[pl.ds(r0, RC), :]
        g = jax.nn.sigmoid(jnp.sum(xc.astype(F32) * gw, axis=-1, keepdims=True))
        hh = _dot(xc, w1_s[...]) + b1
        a = _dot(ot_s[:, pl.ds(r0, RC)].astype(BF16), wo_s[...], TN)
        e = jnp.exp(jnp.minimum(hh, 20.0))
        n = e * (e + 2.0)
        act = (hh * (n / (n + 2.0))).astype(BF16)
        b = _dot(act, w2_s[...])
        out_s[pl.ds(r0, RC), :] = (g * a + (1.0 - g) * b).astype(BF16)
        out_cp(i).start()
        return _

    lax.fori_loop(0, NRC, rows_fn, 0)
    for i in range(NRC):
        out_cp(i).wait()


@jax.jit
def pallas_gated_mix__mha_block__dense_activation_mish__prompt_kernel(
    A_x: jax.Array,
    A_wqkv: jax.Array,
    A_wo: jax.Array,
    B_x: jax.Array,
    B_w1: jax.Array,
    B_b1: jax.Array,
    B_w2: jax.Array,
    gate_w: jax.Array,
):
    del B_x
    hbm = pl.BlockSpec(memory_space=pl.ANY)
    out = pl.pallas_call(
        _kernel,
        out_shape=jax.ShapeDtypeStruct((S, D), A_x.dtype),
        in_specs=[hbm] * 7,
        out_specs=hbm,
        scratch_shapes=[
            pltpu.VMEM((S, D), BF16),
            pltpu.VMEM((D, D), BF16),
            pltpu.VMEM((D, D), BF16),
            pltpu.VMEM((D, D), BF16),
            pltpu.VMEM((D, D), BF16),
            pltpu.VMEM((D, F), BF16),
            pltpu.VMEM((F,), BF16),
            pltpu.VMEM((F, D), BF16),
            pltpu.VMEM((D,), BF16),
            pltpu.VMEM((S, D), BF16),
            pltpu.VMEM((2 * D, D), BF16),
            pltpu.VMEM((2 * NT - 1, S, 128), BF16),
            pltpu.VMEM((D, S), F32),
            pltpu.VMEM((D, S), F32),
            pltpu.VMEM((H, 128, S), BF16),
            pltpu.SemaphoreType.DMA((NXC + 8,)),
            pltpu.SemaphoreType.DMA((NRC,)),
        ],
        compiler_params=pltpu.CompilerParams(vmem_limit_bytes=110 * 1024 * 1024),
    )(A_x.reshape(S, D), A_wqkv, A_wo, B_w1, B_b1, B_w2, gate_w)
    return out.reshape(1, S, D)
```

```python
import jax
import jax.numpy as jnp
from jax import lax
import jax.experimental.pallas as pl
import jax.experimental.pallas.tpu as pltpu

S, D, H, DH, F = 2048, 640, 32, 20, 1536
NT = D // 128
LOG2E = 1.4426950408889634
QSCALE = (DH ** -0.5) * LOG2E
XC = 512
NXC = S // XC
QB, KB, AHEAD = 512, 128, 6
assert XC == QB
RC = 512
NRC = S // RC

F32, BF16, I32 = jnp.float32, jnp.bfloat16, jnp.int32
NN = (((1,), (0,)), ((), ()))
NT_DIMS = (((1,), (1,)), ((), ()))
TN = (((0,), (0,)), ((), ()))


def _dot(a, b, dims=NN):
    return lax.dot_general(a, b, dims, preferred_element_type=F32)


def _kernel(x_hbm, wqkv_hbm, wo_hbm, w1_hbm, b1_hbm, w2_hbm, gw_hbm, o_hbm,
            x_s, wq_s, wk_s, wv_s, wo_s, w1_s, b1_s, w2_s, gw_s, out_s,
            wt_s, k_s, vt_s, ot_s, w_s, in_sem, out_sem):
    def cp(src, dst, i):
        return pltpu.make_async_copy(src, dst, in_sem.at[i])

    x_cp = [cp(x_hbm.at[pl.ds(c * XC, XC), :], x_s.at[pl.ds(c * XC, XC), :], c)
            for c in range(NXC)]
    wq_cp = cp(wqkv_hbm.at[:, pl.ds(0, D)], wq_s, NXC)
    wk_cp = cp(wqkv_hbm.at[:, pl.ds(D, D)], wk_s, NXC + 1)
    wv_cp = cp(wqkv_hbm.at[:, pl.ds(2 * D, D)], wv_s, NXC + 2)
    late = [cp(wo_hbm, wo_s, NXC + 3), cp(w1_hbm, w1_s, NXC + 4), cp(w2_hbm, w2_s, NXC + 5),
            cp(b1_hbm, b1_s, NXC + 6), cp(gw_hbm, gw_s, NXC + 7)]

    def proj_k(c, extra=()):
        rows = pl.ds(c * XC, XC)
        lane = lax.broadcasted_iota(I32, (XC, 128), 1)
        xc = x_s[rows, :]
        rows2 = pl.ds(c * XC // 2, XC // 2)
        k = []
        for t in range(NT):
            parts = 4 if t == NT - 1 else 1
            w = wk_s[:, 128 * t:128 * t + 128]
            k.append(jnp.concatenate(
                [_dot(xc[i * XC // parts:(i + 1) * XC // parts], w) for i in range(parts)],
                axis=0).astype(BF16))
            k_s[t, rows2, :] = pltpu.bitcast(k[t], I32)
            if t:
                k_s[NT + t - 1, rows2, :] = pltpu.bitcast(jnp.where(lane >= 64, k[t - 1], k[t]), I32)
            for fn in extra:
                fn(t)

    def proj_qv(c, good):
        cols = pl.ds(pl.multiple_of(c * XC, XC), XC)
        qv = _dot(wt_s[...], x_s[cols, :], NT_DIMS)
        vt_s[:, cols] = qv[D:].astype(BF16).astype(F32)
        small = jnp.where(jnp.abs(qv[D:]) <= 2.0 ** 50, 1.0, 0.0)
        good = jnp.minimum(good, jnp.min(small, axis=0, keepdims=True))
        r = lax.broadcasted_iota(I32, (16, XC), 0)
        for h in range(H):
            lo, hi = DH * h, DH * h + DH
            for i in range(8):
                g0 = next((g for g in range(lo // 16 * 16, hi, 16) if g % 128 == 16 * i), None)
                if g0 is not None:
                    keep = (r >= lo - g0) & (r < hi - g0)
                    q = jnp.where(keep, qv[g0:g0 + 16] * QSCALE, 0.0)
                    w_s[h, 16 * i:16 * i + 16, cols] = q.astype(BF16)
        return good

    half = NXC // 2
    wk_cp.start()
    x_cp[0].start()
    for h in range(H):
        live = {g % 128 // 16 for g in range(DH * h // 16 * 16, DH * h + DH, 16)}
        for i in range(8):
            if i not in live:
                w_s[h, 16 * i:16 * i + 16, :] = jnp.zeros((16, S), BF16)
    wk_cp.wait()
    x_cp[0].wait()
    for c in range(1, half):
        x_cp[c].start()
    wq_cp.start()
    wv_cp.start()
    for c in range(half, NXC):
        x_cp[c].start()
    proj_k(0)
    for c in range(1, half):
        x_cp[c].wait()
        proj_k(c)
    wq_cp.wait()
    wv_cp.wait()
    for c in range(half, NXC):
        x_cp[c].wait()
    for c in late:
        c.start()
    slabs = [(w, r, t) for w, r in ((wq_s, 0), (wv_s, D)) for t in range(NT)]

    def transpose_slab(i):
        w, r, t = slabs[i]
        wt_s[r + 128 * t:r + 128 * t + 128, :] = w[:, 128 * t:128 * t + 128].T

    for c in range(half, NXC):
        proj_k(c, [lambda t, c=c: transpose_slab((c - half) * NT + t)])
    good = lax.fori_loop(0, NXC, proj_qv, jnp.ones((1, XC), F32))

    def head_fns(i, u):
        h = i * 2 + u
        c = h * DH
        t = c // 128
        kidx = jnp.where(c - t * 128 + DH > 128, NT + t, t)
        g8 = pl.multiple_of(i * (2 * DH) + u * 16, 8)
        lrow = 0 if u else DH
        row = lax.broadcasted_iota(I32, (24, KB), 0)
        row8 = lax.broadcasted_iota(I32, (8, QB), 0)

        def qk(g, j):
            return _dot(pltpu.bitcast(k_s[kidx, pl.ds(j * KB // 2, KB // 2), :], BF16), w_s[h, :, pl.ds(g * QB, QB)])

        def vt(j):
            return jnp.where(row == lrow, 1.0, vt_s[pl.ds(g8, 24), pl.ds(j * KB, KB)])

        def finish(g, acc, good):
            cols = pl.ds(g * QB, QB)
            l = acc[lrow:lrow + 1]
            r = pl.reciprocal(l, approx=True)
            o = acc * (r * (2.0 - l * r))
            if u:
                ot_s[pl.ds(g8, 8), cols] = jnp.where(row8 >= 4, o[:8], ot_s[pl.ds(g8, 8), cols])
                ot_s[pl.ds(g8 + 8, 16), cols] = o[8:]
            else:
                ot_s[pl.ds(g8, 24), cols] = o
            return jnp.minimum(good, jnp.where((l >= 2.0 ** -60) & (l <= 2.0 ** 60), 1.0, 0.0))

        return qk, vt, finish

    def heads_fast(i, good):
        fns = [head_fns(i, u) for u in range(2)]
        segs = [(u, g, j) for u in range(2) for g in range(S // QB) for j in range(S // KB)]
        pend = [fns[u][0](g, j) for u, g, j in segs[:AHEAD]]
        acc = None
        for n, (u, g, j) in enumerate(segs):
            if n + AHEAD < len(segs):
                u2, g2, j2 = segs[n + AHEAD]
                pend.append(fns[u2][0](g2, j2))
            d = _dot(fns[u][1](j), jnp.exp2(pend.pop(0)).astype(BF16))
            acc = d if j == 0 else acc + d
            if j == S // KB - 1:
                good = fns[u][2](g, acc, good)
        return good

    def tile_true_max(i, _):
        h = i // (S // 128)
        q0 = pl.multiple_of((i % (S // 128)) * 128, 128)
        c = h * DH
        t = c // 128
        kidx = jnp.where(c - t * 128 + DH > 128, NT + t, t)
        g8 = pl.multiple_of((c // 8) * 8, 8)
        o = c - g8
        lrow = jnp.where(o == 0, DH, 0)
        row = lax.broadcasted_iota(I32, (24, 128), 0)

        def qk(j):
            k0 = pl.multiple_of(j * (KB // 2), KB // 2)
            return _dot(pltpu.bitcast(k_s[kidx, pl.ds(k0, KB // 2), :], BF16), w_s[h, :, pl.ds(q0, 128)])

        m = lax.fori_loop(
            0, S // KB, lambda j, m: jnp.maximum(m, jnp.max(qk(j), axis=0, keepdims=True)),
            jnp.full((1, 128), -jnp.inf, F32))

        def pv(j, acc):
            v = vt_s[pl.ds(g8, 24), pl.ds(pl.multiple_of(j * KB, KB), KB)]
            return acc + _dot(jnp.where(row == lrow, 1.0, v), jnp.exp2(qk(j) - m).astype(BF16))

        acc = lax.fori_loop(0, S // KB, pv, jnp.zeros((24, 128), F32))
        l = jnp.sum(jnp.where(row == lrow, acc, 0.0), axis=0, keepdims=True)
        keep = (row >= o) & (row < o + DH)
        dst = ot_s.at[pl.ds(g8, 24), pl.ds(q0, 128)]
        dst[...] = jnp.where(keep, acc * (1.0 / l), dst[...])
        return _

    good = lax.fori_loop(0, H // 2, heads_fast, good)

    @pl.when(jnp.min(good) < 0.5)
    def _():
        lax.fori_loop(0, H * (S // 128), tile_true_max, 0)

    for c in late:
        c.wait()
    gw = gw_s[...].reshape(1, D).astype(F32)
    b1 = b1_s[...].reshape(1, F).astype(F32)

    def out_cp(i):
        rows = pl.ds(pl.multiple_of(i * RC, RC), RC)
        return pltpu.make_async_copy(out_s.at[rows, :], o_hbm.at[rows, :], out_sem.at[i])

    def rows_fn(i, _):
        r0 = pl.multiple_of(i * RC, RC)
        xc = x_s[pl.ds(r0, RC), :]
        g = jax.nn.sigmoid(jnp.sum(xc.astype(F32) * gw, axis=-1, keepdims=True))
        hh = _dot(xc, w1_s[...]) + b1
        a = _dot(ot_s[:, pl.ds(r0, RC)].astype(BF16), wo_s[...], TN)
        e = jnp.exp(jnp.minimum(hh, 20.0))
        n = e * (e + 2.0)
        act = (hh * (n / (n + 2.0))).astype(BF16)
        b = _dot(act, w2_s[...])
        out_s[pl.ds(r0, RC), :] = (g * a + (1.0 - g) * b).astype(BF16)
        out_cp(i).start()
        return _

    lax.fori_loop(0, NRC, rows_fn, 0)
    for i in range(NRC):
        out_cp(i).wait()


@jax.jit
def pallas_gated_mix__mha_block__dense_activation_mish__prompt_kernel(
    A_x: jax.Array,
    A_wqkv: jax.Array,
    A_wo: jax.Array,
    B_x: jax.Array,
    B_w1: jax.Array,
    B_b1: jax.Array,
    B_w2: jax.Array,
    gate_w: jax.Array,
):
    del B_x
    hbm = pl.BlockSpec(memory_space=pl.ANY)
    out = pl.pallas_call(
        _kernel,
        out_shape=jax.ShapeDtypeStruct((S, D), A_x.dtype),
        in_specs=[hbm] * 7,
        out_specs=hbm,
        scratch_shapes=[
            pltpu.VMEM((S, D), BF16),
            pltpu.VMEM((D, D), BF16),
            pltpu.VMEM((D, D), BF16),
            pltpu.VMEM((D, D), BF16),
            pltpu.VMEM((D, D), BF16),
            pltpu.VMEM((D, F), BF16),
            pltpu.VMEM((F,), BF16),
            pltpu.VMEM((F, D), BF16),
            pltpu.VMEM((D,), BF16),
            pltpu.VMEM((S, D), BF16),
            pltpu.VMEM((2 * D, D), BF16),
            pltpu.VMEM((2 * NT - 1, S // 2, 128), I32),
            pltpu.VMEM((D, S), F32),
            pltpu.VMEM((D, S), F32),
            pltpu.VMEM((H, 128, S), BF16),
            pltpu.SemaphoreType.DMA((NXC + 8,)),
            pltpu.SemaphoreType.DMA((NRC,)),
        ],
        compiler_params=pltpu.CompilerParams(vmem_limit_bytes=110 * 1024 * 1024),
    )(A_x.reshape(S, D), A_wqkv, A_wo, B_w1, B_b1, B_w2, gate_w)
    return out.reshape(1, S, D)
```
